```python
import os as _os
_os.environ.setdefault("JAX_PLATFORMS", "cpu")
import jax
import jax.numpy as jnp

def _softmax(x, axis=-1):
    return jax.nn.softmax(x, axis=axis)
def _gelu(x):
    return jax.nn.gelu(x, approximate=True)
def _silu(x):
    return jax.nn.silu(x)
def _sigmoid(x):
    return jax.nn.sigmoid(x)
def _layernorm(x, axis=-1, eps=1e-5):
    m = jnp.mean(x, axis=axis, keepdims=True)
    v = jnp.var(x, axis=axis, keepdims=True)
    return (x - m) / jnp.sqrt(v + eps)
def _scatter_add(tgt, idx, src, axis=0):
    return tgt.at[idx].add(src)
def _segment_sum(src, seg, n):
    return jax.ops.segment_sum(src, seg, n)
class _Rng:
    def __init__(self, key):
        self._k = key
    def _next(self):
        self._k, sub = jax.random.split(self._k)
        return sub
    def normal(self, shape):
        return jax.random.normal(self._next(), shape, dtype=jnp.bfloat16)
    def randint(self, lo, hi, shape):
        return jax.random.randint(self._next(), shape, lo, hi, dtype=jnp.int32)
    def uniform(self, shape, lo=0.0, hi=1.0):
        return jax.random.uniform(self._next(), shape, jnp.bfloat16, lo, hi)
    def permutation(self, n):
        return jax.random.permutation(self._next(), n)


kernel_name = 'standalone__gqa_softmax__near_ridge'

def setup_inputs():
    _rng = _Rng(jax.random.key(int.from_bytes(__import__("os").urandom(4), "little")))
    _w = (lambda a: (lambda t: t.astype(jnp.bfloat16) if jnp.issubdtype(t.dtype, jnp.floating) else t)(jnp.asarray(a)))
    B, Hq, Hkv, Sq, Sk, D = 8, 32, 8, 112, 2048, 128
    return {
        "q": _w((lambda *s: _rng.normal(s) * 0.4)(B, Hq, Sq, D)),
        "k": _w((lambda *s: _rng.normal(s) * 0.4)(B, Hkv, Sk, D)),
        "v": _w((lambda *s: _rng.normal(s) * 0.05)(B, Hkv, Sk, D)),
    }

def reference(q, k, v):
    B, Hq, Sq, D = q.shape
    Hkv = k.shape[1]
    rep = Hq // Hkv
    k = jnp.repeat(k, rep, axis=1)
    v = jnp.repeat(v, rep, axis=1)
    scale = D ** -0.5
    scores = jnp.einsum("bhqd,bhkd->bhqk", q, k) * scale
    p = _softmax(scores, axis=-1)
    return jnp.einsum("bhqk,bhkd->bhqd", p, v)
```

```python
import jax
import jax.numpy as jnp
import jax.experimental.pallas as pl
import jax.experimental.pallas.tpu as pltpu

_LOG2E = 1.4426950408889634
_CHUNK = 512


def _kernel(q_ref, k_ref, v_ref, o_ref):
    q = q_ref[0]
    c = q.shape[-1] ** -0.5 * _LOG2E
    m = l = acc = None
    for j in range(k_ref.shape[1] // _CHUNK):
        kj = k_ref[0, j * _CHUNK:(j + 1) * _CHUNK, :]
        vj = v_ref[0, j * _CHUNK:(j + 1) * _CHUNK, :]
        s = jax.lax.dot_general(q, kj, (((1,), (1,)), ((), ())), preferred_element_type=jnp.float32)
        mj = jnp.max(s, axis=-1, keepdims=True)
        mn = mj if j == 0 else jnp.maximum(m, mj)
        p = jnp.exp2((s - mn) * c)
        lj = jnp.sum(p, axis=-1, keepdims=True)
        oj = jnp.dot(p.astype(jnp.bfloat16), vj, preferred_element_type=jnp.float32)
        if j == 0:
            l, acc = lj, oj
        else:
            a = jnp.exp2((m - mn) * c)
            l = a * l + lj
            acc = a * acc + oj
        m = mn
    o_ref[0] = (acc / l).astype(o_ref.dtype)


@jax.jit
def pallas_standalone__gqa_softmax__near_ridge_kernel(q: jax.Array, k: jax.Array, v: jax.Array):
    B, Hq, Sq, D = q.shape
    _, Hkv, Sk, _ = k.shape
    R = (Hq // Hkv) * Sq
    N = B * Hkv
    out = pl.pallas_call(
        _kernel,
        grid=(N,),
        in_specs=[
            pl.BlockSpec((1, R, D), lambda i: (i, 0, 0)),
            pl.BlockSpec((1, Sk, D), lambda i: (i, 0, 0)),
            pl.BlockSpec((1, Sk, D), lambda i: (i, 0, 0)),
        ],
        out_specs=pl.BlockSpec((1, R, D), lambda i: (i, 0, 0)),
        out_shape=jax.ShapeDtypeStruct((N, R, D), q.dtype),
        compiler_params=pltpu.CompilerParams(dimension_semantics=("parallel",)),
    )(q.reshape(N, R, D), k.reshape(N, Sk, D), v.reshape(N, Sk, D))
    return out.reshape(B, Hq, Sq, D)
```

```python
import numpy as np
import jax
import jax.numpy as jnp
from jax import lax
import jax.experimental.pallas as pl
import jax.experimental.pallas.tpu as pltpu

_LOG2E = 1.4426950408889634
_NT = (((1,), (1,)), ((), ()))
_RB = 64
_PK = 512
_XLAG = 2
_U = 4
_RAMP = (1, 1, 2)
_NS = 16


def _tiles(x):
    return [x[:, u * 128:(u + 1) * 128] for u in range(x.shape[1] // 128)]


def _tree(f, xs):
    xs = list(xs)
    while len(xs) > 1:
        xs = [f(xs[i], xs[i + 1]) if i + 1 < len(xs) else xs[i] for i in range(0, len(xs), 2)]
    return xs[0]


def _make_kernel(N, R, SK, D):
    f32, bf16 = jnp.float32, jnp.bfloat16
    npi, nrb = SK // _PK, R // _RB
    T = npi * nrb
    lag = npi + _XLAG
    c = D ** -0.5 * _LOG2E
    n0 = sum(_RAMP)
    niter = (N - n0) // _U
    assert R % _RB == 0 and SK % _PK == 0 and D == 128
    assert (N - n0) % _U == 0 and n0 % _U == 0 and _NS % _U == 0 and niter >= 2

    live = [(("s", t), _PK) for t in range(-lag, 0)] + [(("m", u), 128) for u in range(-lag // npi, 0)]
    if lag % npi:
        live += [("l", 128), ("acc", 128)]

    def kern(zero_ref, q_hbm, k_hbm, v_hbm, o_hbm, qb, kb, vb, ob, sq, sk, sv, so, *carry):
        st, hist = {}, []
        keep = jnp.full((_RB, 128), zero_ref[0], jnp.int32) == 0

        def weights(ref, slot, j):
            w = ref.bitcast(jnp.uint32)[slot, j * _PK // 2:(j + 1) * _PK // 2, :]
            return pltpu.bitcast(w, bf16)

        def qk(nb, t):
            u, j = divmod(t, npi)
            dn, rb = divmod(u, nrb)
            slot = (nb + dn) % _NS
            if j == 0:
                st["q"] = (qb[slot, rb * _RB:(rb + 1) * _RB, :].astype(f32) * c).astype(bf16)
            s = lax.dot_general(st["q"], weights(kb, slot, j), _NT, preferred_element_type=f32)
            st[("s", t)] = s
            el = _tree(jnp.maximum, _tiles(s))
            st["mx"] = el if j == 0 else jnp.maximum(st["mx"], el)
            if j == npi - 1:
                st[("m", u)] = jnp.broadcast_to(jnp.max(st.pop("mx"), axis=-1, keepdims=True), (_RB, 128))
                st.pop("q")

        def pv(nb, t):
            u, j = divmod(t, npi)
            dn, rb = divmod(u, nrb)
            slot = (nb + dn) % _NS
            m = st[("m", u)]
            if len(hist) > 1:
                m = jnp.where(keep, m, hist.pop(0))
            p = jnp.exp2(st.pop(("s", t)) - jnp.concatenate([m] * (_PK // 128), axis=1))
            lj = _tree(jnp.add, _tiles(p))
            oj = jnp.dot(p.astype(bf16), weights(vb, slot, j), preferred_element_type=f32)
            st["l"] = lj if j == 0 else st["l"] + lj
            st["acc"] = oj if j == 0 else st["acc"] + oj
            if j == npi - 1:
                st.pop(("m", u))
                l = jnp.sum(st.pop("l"), axis=-1, keepdims=True)
                o = st.pop("acc") * (1.0 / l)
                ob[nb + dn, rb * _RB:(rb + 1) * _RB, :] = o.astype(bf16)
                hist.append(o)
            else:
                hist.append(st["acc"])

        def run(nb, t0, t1, do_qk=True, skip_neg_pv=False):
            for t in range(t0, t1):
                if do_qk:
                    qk(nb, t + lag)
                if not (skip_neg_pv and t < 0):
                    pv(nb, t)

        def save(shift):
            for (k, _), ref in zip(live, carry):
                if isinstance(k, tuple):
                    k = (k[0], k[1] + (shift if k[0] == "s" else shift // npi))
                ref[...] = st.pop(k)
            assert not st
            hist.clear()

        def load():
            for (k, _), ref in zip(live, carry):
                st[k] = ref[...]

        def fetch(n, u, e):
            src, dst = pl.ds(n, u), pl.ds(n % _NS, u)
            return (pltpu.make_async_copy(q_hbm.at[src], qb.at[dst], sq.at[e]),
                    pltpu.make_async_copy(k_hbm.at[src], kb.at[dst], sk.at[e]),
                    pltpu.make_async_copy(v_hbm.at[src], vb.at[dst], sv.at[e]))

        def put(n, u):
            return pltpu.make_async_copy(ob.at[pl.ds(n, u)], o_hbm.at[pl.ds(n, u)], so.at[0])

        segs = [(sum(_RAMP[:i]), u) for i, u in enumerate(_RAMP)] + [(n0, _U), (n0 + _U, _U)]
        for x in fetch(*segs[0], 0):
            x.start()
        for i, (n, u) in enumerate(segs[:-2]):
            for x in fetch(n, u, i % 2):
                x.wait()
            if i == 0:
                for x in fetch(*segs[1], 1):
                    x.start()
            else:
                load()
            run(n, -lag, u * T - lag, skip_neg_pv=(i == 0))
            save(u * T)
            for x in fetch(*segs[i + 2], i % 2):
                x.start()
        put(0, n0 - 1).start()

        def segment(i, prefetch):
            n = n0 + i * _U
            e = (len(_RAMP) + i) % 2
            for x in fetch(n, _U, e):
                x.wait()
            load()
            run(n, -lag, _U * T - lag)
            save(_U * T)
            if prefetch:
                for x in fetch(n + 2 * _U, _U, e):
                    x.start()
            put(n - 1, _U).start()
            return 0

        lax.fori_loop(0, niter - 2, lambda i, _: segment(i, True), 0)
        lax.fori_loop(niter - 2, niter, lambda i, _: segment(i, False), 0)
        load()
        run(N, -lag, 0, do_qk=False)
        put(N - 1, 1).start()
        put(0, N).wait()

    scratch = [pltpu.VMEM((_NS, R, D), bf16), pltpu.VMEM((_NS, SK, D), bf16), pltpu.VMEM((_NS, SK, D), bf16),
               pltpu.VMEM((N, R, D), bf16),
               pltpu.SemaphoreType.DMA((2,)), pltpu.SemaphoreType.DMA((2,)), pltpu.SemaphoreType.DMA((2,)),
               pltpu.SemaphoreType.DMA((1,))] + [pltpu.VMEM((_RB, w), f32) for _, w in live]
    return kern, scratch


@jax.jit
def pallas_standalone__gqa_softmax__near_ridge_kernel(q: jax.Array, k: jax.Array, v: jax.Array):
    B, Hq, Sq, D = q.shape
    _, Hkv, Sk, _ = k.shape
    R = (Hq // Hkv) * Sq
    N = B * Hkv
    kern, scratch = _make_kernel(N, R, Sk, D)
    hbm = pl.BlockSpec(memory_space=pl.ANY)
    out = pl.pallas_call(
        kern,
        in_specs=[pl.BlockSpec(memory_space=pltpu.SMEM), hbm, hbm, hbm],
        out_specs=hbm,
        out_shape=jax.ShapeDtypeStruct((N, R, D), q.dtype),
        scratch_shapes=scratch,
        compiler_params=pltpu.CompilerParams(vmem_limit_bytes=100 * 1024 * 1024),
    )(np.zeros((1,), np.int32), q.reshape(N, R, D), k.reshape(N, Sk, D), v.reshape(N, Sk, D))
    return out.reshape(B, Hq, Sq, D)
```

```python
import numpy as np
import jax
import jax.numpy as jnp
from jax import lax
import jax.experimental.pallas as pl
import jax.experimental.pallas.tpu as pltpu

_LOG2E = 1.4426950408889634
_NT = (((1,), (1,)), ((), ()))
_RB = 64
_PK = 512
_XLAG = 2
_U = 4
_RAMP = (1, 1, 2, 2, 2)
_NS = 16


def _tiles(x):
    return [x[:, u * 128:(u + 1) * 128] for u in range(x.shape[1] // 128)]


def _tree(f, xs):
    xs = list(xs)
    while len(xs) > 1:
        xs = [f(xs[i], xs[i + 1]) if i + 1 < len(xs) else xs[i] for i in range(0, len(xs), 2)]
    return xs[0]


def _make_kernel(N, R, SK, D):
    f32, bf16 = jnp.float32, jnp.bfloat16
    npi, nrb = SK // _PK, R // _RB
    T = npi * nrb
    lag = npi + _XLAG
    c = D ** -0.5 * _LOG2E
    n0 = sum(_RAMP)
    niter = (N - n0) // _U
    assert R % _RB == 0 and SK % _PK == 0 and D == 128
    assert (N - n0) % _U == 0 and n0 % _U == 0 and _NS % _U == 0 and niter >= 2
    assert _NS & (_NS - 1) == 0 and n0 + 2 * _U <= _NS and 2 * _U + 1 <= _NS

    live = [(("s", t), _PK) for t in range(-lag, 0)] + [(("m", u), 128) for u in range(-lag // npi, 0)]
    if lag % npi:
        live += [("l", 128), ("acc", 128)]

    def kern(zero_ref, q_hbm, k_hbm, v_hbm, o_hbm, qb, kb, vb, ob, sq, sk, sv, so, *carry):
        st, hist = {}, []
        keep = jnp.full((_RB, 128), zero_ref[0], jnp.int32) == 0

        def weights(ref, slot, j):
            return ref[slot, j * _PK:(j + 1) * _PK, :]

        def qk(nb, t):
            u, j = divmod(t, npi)
            dn, rb = divmod(u, nrb)
            slot = (nb + dn) & (_NS - 1)
            if j == 0:
                st["q"] = (qb[slot, rb * _RB:(rb + 1) * _RB, :].astype(f32) * c).astype(bf16)
            s = lax.dot_general(st["q"], weights(kb, slot, j), _NT, preferred_element_type=f32)
            st[("s", t)] = s
            el = _tree(jnp.maximum, _tiles(s))
            st["mx"] = el if j == 0 else jnp.maximum(st["mx"], el)
            if j == npi - 1:
                st[("m", u)] = jnp.broadcast_to(jnp.max(st.pop("mx"), axis=-1, keepdims=True), (_RB, 128))
                st.pop("q")

        def pv(nb, t):
            u, j = divmod(t, npi)
            dn, rb = divmod(u, nrb)
            slot = (nb + dn) & (_NS - 1)
            m = st[("m", u)]
            if len(hist) > 1:
                m = jnp.where(keep, m, hist.pop(0))
            p = jnp.exp2(st.pop(("s", t)) - jnp.concatenate([m] * (_PK // 128), axis=1))
            lj = _tree(jnp.add, _tiles(p))
            oj = jnp.dot(p.astype(bf16), weights(vb, slot, j), preferred_element_type=f32)
            st["l"] = lj if j == 0 else st["l"] + lj
            st["acc"] = oj if j == 0 else st["acc"] + oj
            if j == npi - 1:
                st.pop(("m", u))
                l = jnp.sum(st.pop("l"), axis=-1, keepdims=True)
                o = st.pop("acc") * (1.0 / l)
                ob[nb + dn, rb * _RB:(rb + 1) * _RB, :] = o.astype(bf16)
                hist.append(o)
            else:
                hist.append(st["acc"])

        def run(nb, t0, t1, do_qk=True, skip_neg_pv=False):
            for t in range(t0, t1):
                if do_qk:
                    qk(nb, t + lag)
                if not (skip_neg_pv and t < 0):
                    pv(nb, t)

        def save(shift):
            for (k, _), ref in zip(live, carry):
                if isinstance(k, tuple):
                    k = (k[0], k[1] + (shift if k[0] == "s" else shift // npi))
                ref[...] = st.pop(k)
            assert not st
            hist.clear()

        def load():
            for (k, _), ref in zip(live, carry):
                st[k] = ref[...]

        def fetch(n, u, e):
            src, dst = pl.ds(n, u), pl.ds(n & (_NS - 1), u)
            return (pltpu.make_async_copy(q_hbm.at[src], qb.at[dst], sq.at[e]),
                    pltpu.make_async_copy(k_hbm.at[src], kb.at[dst], sk.at[e]),
                    pltpu.make_async_copy(v_hbm.at[src], vb.at[dst], sv.at[e]))

        def put(n, u):
            return pltpu.make_async_copy(ob.at[pl.ds(n, u)], o_hbm.at[pl.ds(n, u)], so.at[0])

        segs = [(sum(_RAMP[:i]), u) for i, u in enumerate(_RAMP)]
        for i, (n, u) in enumerate(segs):
            for x in fetch(n, u, 2 + i):
                x.start()
        for e in (0, 1):
            for x in fetch(n0 + e * _U, _U, e):
                x.start()
        for i, (n, u) in enumerate(segs):
            for x in fetch(n, u, 2 + i):
                x.wait()
            if i:
                load()
            run(n, -lag, u * T - lag, skip_neg_pv=(i == 0))
            save(u * T)
        put(0, n0 - 1).start()

        def segment(i, prefetch):
            n = n0 + i * _U
            e = i % 2
            for x in fetch(n, _U, e):
                x.wait()
            load()
            run(n, -lag, _U * T - lag)
            save(_U * T)
            if prefetch:
                for x in fetch(n + 2 * _U, _U, e):
                    x.start()
            put(n - 1, _U).start()
            return 0

        lax.fori_loop(0, niter - 2, lambda i, _: segment(i, True), 0)
        lax.fori_loop(niter - 2, niter, lambda i, _: segment(i, False), 0)
        load()
        run(N, -lag, 0, do_qk=False)
        put(N - 1, 1).start()
        put(0, N).wait()

    scratch = [pltpu.VMEM((_NS, R, D), bf16), pltpu.VMEM((_NS, SK, D), bf16), pltpu.VMEM((_NS, SK, D), bf16),
               pltpu.VMEM((N, R, D), bf16),
               pltpu.SemaphoreType.DMA((2 + len(_RAMP),)), pltpu.SemaphoreType.DMA((2 + len(_RAMP),)), pltpu.SemaphoreType.DMA((2 + len(_RAMP),)),
               pltpu.SemaphoreType.DMA((1,))] + [pltpu.VMEM((_RB, w), f32) for _, w in live]
    return kern, scratch


@jax.jit
def pallas_standalone__gqa_softmax__near_ridge_kernel(q: jax.Array, k: jax.Array, v: jax.Array):
    B, Hq, Sq, D = q.shape
    _, Hkv, Sk, _ = k.shape
    R = (Hq // Hkv) * Sq
    N = B * Hkv
    kern, scratch = _make_kernel(N, R, Sk, D)
    hbm = pl.BlockSpec(memory_space=pl.ANY)
    out = pl.pallas_call(
        kern,
        in_specs=[pl.BlockSpec(memory_space=pltpu.SMEM), hbm, hbm, hbm],
        out_specs=hbm,
        out_shape=jax.ShapeDtypeStruct((N, R, D), q.dtype),
        scratch_shapes=scratch,
        compiler_params=pltpu.CompilerParams(vmem_limit_bytes=100 * 1024 * 1024),
    )(np.zeros((1,), np.int32), q.reshape(N, R, D), k.reshape(N, Sk, D), v.reshape(N, Sk, D))
    return out.reshape(B, Hq, Sq, D)
```
